```python
import os as _os
_os.environ.setdefault("JAX_PLATFORMS", "cpu")
import jax
import jax.numpy as jnp

def _softmax(x, axis=-1):
    return jax.nn.softmax(x, axis=axis)
def _gelu(x):
    return jax.nn.gelu(x, approximate=True)
def _silu(x):
    return jax.nn.silu(x)
def _sigmoid(x):
    return jax.nn.sigmoid(x)
def _layernorm(x, axis=-1, eps=1e-5):
    m = jnp.mean(x, axis=axis, keepdims=True)
    v = jnp.var(x, axis=axis, keepdims=True)
    return (x - m) / jnp.sqrt(v + eps)
def _scatter_add(tgt, idx, src, axis=0):
    return tgt.at[idx].add(src)
def _segment_sum(src, seg, n):
    return jax.ops.segment_sum(src, seg, n)
class _Rng:
    def __init__(self, key):
        self._k = key
    def _next(self):
        self._k, sub = jax.random.split(self._k)
        return sub
    def normal(self, shape):
        return jax.random.normal(self._next(), shape, dtype=jnp.bfloat16)
    def randint(self, lo, hi, shape):
        return jax.random.randint(self._next(), shape, lo, hi, dtype=jnp.int32)
    def uniform(self, shape, lo=0.0, hi=1.0):
        return jax.random.uniform(self._next(), shape, jnp.bfloat16, lo, hi)
    def permutation(self, n):
        return jax.random.permutation(self._next(), n)


kernel_name = 'concat_heads__grouped_kv_mqa__sliding_block__prompt'

def setup_inputs():
    _rng = _Rng(jax.random.key(int.from_bytes(__import__("os").urandom(4), "little")))
    _w = (lambda a: (lambda t: t.astype(jnp.bfloat16) if jnp.issubdtype(t.dtype, jnp.floating) else t)(jnp.asarray(a)))
    def _A_setup():
        B, S, D, H = 1, 2048, 1024, 32
        Dh = D // H
        return {
            "x": _w((lambda *s: _rng.normal(s) * 0.05)(B, S, D)),
            "wq": _w((lambda *s: _rng.normal(s) * 1.6)(D, H * Dh)),
            "wk": _w((lambda *s: _rng.normal(s) * 1.6)(D, Dh)),
            "wv": _w((lambda *s: _rng.normal(s) * 0.1)(D, Dh)),
            "wo": _w((lambda *s: _rng.normal(s) * 0.1)(H * Dh, D)),
        }
    _A_in = _A_setup()

    def _B_setup():
        B, S, D = 1, 2048, 1024
        return {
            "x": _w((lambda *s: _rng.normal(s) * 0.2)(B, S, D)),
            "wqkv": _w((lambda *s: _rng.normal(s) * 0.2)(D, 3 * D)),
            "wo": _w((lambda *s: _rng.normal(s) * 0.05)(D, D)),
        }
    _B_in = _B_setup()

    return {
        "A_x": _A_in["x"],
        "A_wq": _A_in["wq"],
        "A_wk": _A_in["wk"],
        "A_wv": _A_in["wv"],
        "A_wo": _A_in["wo"],
        "B_x": _B_in["x"],
        "B_wqkv": _B_in["wqkv"],
        "B_wo": _B_in["wo"],
    }

def reference(A_x, A_wq, A_wk, A_wv, A_wo, B_x, B_wqkv, B_wo):
    def _A_ref(x, wq, wk, wv, wo):
        B, S, D = x.shape
        H = 32
        Dh = D // H
        q = (lambda x, *d: x.transpose(*d))((x @ wq).reshape(B, S, H, Dh), 0, 2, 1, 3)
        k = x @ wk
        v = x @ wv
        scores = jnp.einsum("bhqd,bkd->bhqk", q, k) * (Dh ** -0.5)
        p = _softmax(scores, axis=-1)
        o = jnp.einsum("bhqk,bkd->bhqd", p, v)
        return (lambda x, *d: x.transpose(*d))(o, 0, 2, 1, 3).reshape(B, S, H * Dh) @ wo

    def _B_ref(x, wqkv, wo):
        B, S, D = x.shape
        H = 32; Dh = D // H; W = 256
        qkv = (lambda x, *d: x.transpose(*d))((x @ wqkv).reshape(B, S, 3, H, Dh), 2, 0, 3, 1, 4)
        q, k, v = qkv[0], qkv[1], qkv[2]
        scores = jnp.einsum("bhqd,bhkd->bhqk", q, k) * (Dh ** -0.5)
        idx = jnp.arange(S)
        mask = (idx[:, None] - idx[None, :] >= 0) & (idx[:, None] - idx[None, :] < W)
        scores = jnp.where(mask[None, None], scores, -1e9)
        p = _softmax(scores, axis=-1)
        o = jnp.einsum("bhqk,bhkd->bhqd", p, v)
        return (lambda x, *d: x.transpose(*d))(o, 0, 2, 1, 3).reshape(B, S, D) @ wo

    a = _A_ref(A_x, A_wq, A_wk, A_wv, A_wo)
    b = _B_ref(B_x, B_wqkv, B_wo)
    return jnp.concatenate([a, b], axis=-1)
```

```python
import math

import jax
import jax.numpy as jnp
import jax.experimental.pallas as pl
import jax.experimental.pallas.tpu as pltpu

S = 2048
D = 1024
H = 32
DH = 32
W = 256
NQ = 512
CK = 128
RC = 512
QB = 128
KB = W + QB
NEG = -1e30
QSCALE = (DH ** -0.5) * math.log2(math.e)

f32 = jnp.float32
bf16 = jnp.bfloat16


def _nt(a, b):
    return jax.lax.dot_general(a, b, (((1,), (1,)), ((), ())),
                               preferred_element_type=f32)


def _nn(a, b):
    return jnp.dot(a, b, preferred_element_type=f32)


def _tree(x, op):
    while x.shape[0] > 8:
        h = x.shape[0] // 2
        x = op(x[:h], x[h:])
    return x


def _kernel(ax_hbm, awq_hbm, awk_hbm, awv_hbm, awo_hbm, bx_hbm, bwqkv_hbm, bwo_hbm,
            out_hbm,
            ax, awq, awk, awv, awo, bx, bwqkv, bwo,
            wkv, kpad, vt_a, q_s, ot_s, s_a, s_b, m_a, m_b,
            kb_s, vtb_s, out_a, out_b,
            in_sems, out_sems):
    srcs = (ax_hbm, awk_hbm, awv_hbm, awq_hbm, bx_hbm, bwqkv_hbm, awo_hbm, bwo_hbm)
    dsts = (ax, awk, awv, awq, bx, bwqkv, awo, bwo)
    copies = [pltpu.make_async_copy(s, d, in_sems.at[i])
              for i, (s, d) in enumerate(zip(srcs, dsts))]
    for c in copies:
        c.start()

    copies[0].wait()
    copies[1].wait()
    copies[2].wait()
    wkv[...] = jnp.zeros(wkv.shape, bf16)
    wkv[:, 0:DH] = awk[...]
    wkv[:, DH:2 * DH] = awv[...]
    lane = jax.lax.broadcasted_iota(jnp.int32, (RC, 128), 1)
    for r in range(S // RC):
        rows = slice(r * RC, (r + 1) * RC)
        kv = _nn(ax[rows, :], wkv[...])
        k_only = jnp.where(lane < DH, kv, 0.0)
        kpad[0, rows, :] = k_only.astype(bf16)
        for j in range(1, 4):
            kpad[j, rows, :] = pltpu.roll(k_only, j * DH, 1).astype(bf16)
        vt_a[:, rows] = kv.T[DH:2 * DH, :].astype(bf16)

    copies[3].wait()
    for r in range(S // RC):
        rows = slice(r * RC, (r + 1) * RC)
        q_s[rows, :] = (_nn(ax[rows, :], awq[...]) * QSCALE).astype(bf16)

    n_units = H * (S // NQ)
    n_ck = S // CK

    def get_q(u):
        t = u // H
        h = u % H
        qg = q_s[pl.ds(pl.multiple_of(t * NQ, NQ), NQ),
                 pl.ds(pl.multiple_of((h // 4) * 128, 128), 128)]
        return qg, h % 4

    def qk_chunk(qg, j, s_ref, c, m8):
        s = _nt(kpad[j, c * CK:(c + 1) * CK, :], qg)
        s_ref[c * CK:(c + 1) * CK, :] = s
        t = _tree(s, jnp.maximum)
        return t if m8 is None else jnp.maximum(m8, t)

    def sm_chunk(s_ref, c, m, l8, acc):
        p = jnp.exp2(s_ref[c * CK:(c + 1) * CK, :] - m)
        t = _tree(p, jnp.add)
        l8 = t if l8 is None else l8 + t
        o = _nn(vt_a[:, c * CK:(c + 1) * CK], p.astype(bf16))
        acc = o if acc is None else acc + o
        return l8, acc

    def step(u_next, s_next, m_next, u_cur, s_cur, m_cur):
        qg, j = get_q(u_next)
        m = m_cur[0:1, :]
        m8 = l8 = acc = None
        for c in range(n_ck):
            m8 = qk_chunk(qg, j, s_next, c, m8)
            l8, acc = sm_chunk(s_cur, c, m, l8, acc)
        m_next[...] = jnp.broadcast_to(jnp.max(m8, axis=0, keepdims=True), (8, NQ))
        t = u_cur // H
        h = u_cur % H
        l = jnp.sum(l8, axis=0, keepdims=True)
        ot_s[pl.ds(pl.multiple_of(h * DH, DH), DH),
             pl.ds(pl.multiple_of(t * NQ, NQ), NQ)] = acc / l

    qg0, j0 = get_q(0)
    m8 = None
    for c in range(n_ck):
        m8 = qk_chunk(qg0, j0, s_a, c, m8)
    m_a[...] = jnp.broadcast_to(jnp.max(m8, axis=0, keepdims=True), (8, NQ))

    def a_body(u, carry):
        un = jnp.minimum(u + 1, n_units - 1)

        @pl.when(u % 2 == 0)
        def _():
            step(un, s_b, m_b, u, s_a, m_a)

        @pl.when(u % 2 == 1)
        def _():
            step(un, s_a, m_a, u, s_b, m_b)
        return carry

    jax.lax.fori_loop(0, n_units, a_body, 0)

    copies[6].wait()
    for r in range(S // RC):
        rows = slice(r * RC, (r + 1) * RC)
        o = ot_s[:, rows].T.astype(bf16)
        out_a[rows, :] = _nn(o, awo[...]).astype(bf16)
    out_a_cp = pltpu.make_async_copy(out_a, out_hbm.at[:, 0:D], out_sems.at[0])
    out_a_cp.start()

    copies[4].wait()
    copies[5].wait()
    kb_s[0:W, :] = jnp.zeros((W, D), bf16)
    vtb_s[:, 0:W] = jnp.zeros((D, W), bf16)
    for r in range(S // RC):
        rows = slice(r * RC, (r + 1) * RC)
        prow = slice(W + r * RC, W + (r + 1) * RC)
        xr = bx[rows, :]
        q_s[rows, :] = (_nn(xr, bwqkv[:, 0:D]) * QSCALE).astype(bf16)
        kb_s[prow, :] = _nn(xr, bwqkv[:, D:2 * D]).astype(bf16)
        vtb_s[:, prow] = _nn(xr, bwqkv[:, 2 * D:3 * D]).T.astype(bf16)

    kk = jax.lax.broadcasted_iota(jnp.int32, (KB, 4 * QB), 0)
    qq = jax.lax.broadcasted_iota(jnp.int32, (KB, 4 * QB), 1) % QB
    band = jnp.logical_and(kk > qq, kk <= qq + W)
    lane_q = jax.lax.broadcasted_iota(jnp.int32, (QB, 128), 1) // DH

    def b_body(t, carry):
        q0 = pl.multiple_of(t * QB, QB)
        valid = jnp.logical_and(band, kk >= W - t * QB)
        bias = jnp.where(valid, 0.0, NEG)
        for g in range(H // 4):
            cols = slice(g * 128, (g + 1) * 128)
            qg = q_s[pl.ds(q0, QB), cols]
            qm = jnp.concatenate(
                [jnp.where(lane_q == j, qg, jnp.zeros_like(qg)) for j in range(4)],
                axis=0)
            kg = kb_s[pl.ds(q0, KB), cols]
            s = _nt(kg, qm) + bias
            m = jnp.max(_tree(s, jnp.maximum), axis=0, keepdims=True)
            p = jnp.exp2(s - m)
            l = jnp.sum(_tree(p, jnp.add), axis=0, keepdims=True)
            pb = p.astype(bf16)
            for j in range(4):
                hrow = slice(g * 128 + j * DH, g * 128 + (j + 1) * DH)
                o = _nn(vtb_s[hrow, pl.ds(q0, KB)], pb[:, j * QB:(j + 1) * QB])
                ot_s[hrow, pl.ds(q0, QB)] = o / l[:, j * QB:(j + 1) * QB]
        return carry

    jax.lax.fori_loop(0, S // QB, b_body, 0)

    copies[7].wait()
    out_b_cps = []
    for r in range(S // RC):
        rows = slice(r * RC, (r + 1) * RC)
        o = ot_s[:, rows].T.astype(bf16)
        out_b[rows, :] = _nn(o, bwo[...]).astype(bf16)
        cp = pltpu.make_async_copy(out_b.at[rows, :], out_hbm.at[rows, D:2 * D],
                                   out_sems.at[1 + r])
        cp.start()
        out_b_cps.append(cp)
    out_a_cp.wait()
    for cp in out_b_cps:
        cp.wait()


@jax.jit
def pallas_concat_heads__grouped_kv_mqa__sliding_block__prompt_kernel(
    A_x: jax.Array,
    A_wq: jax.Array,
    A_wk: jax.Array,
    A_wv: jax.Array,
    A_wo: jax.Array,
    B_x: jax.Array,
    B_wqkv: jax.Array,
    B_wo: jax.Array,
):
    ax = A_x.reshape(S, D)
    bx = B_x.reshape(S, D)
    any_spec = pl.BlockSpec(memory_space=pl.ANY)
    out = pl.pallas_call(
        _kernel,
        out_shape=jax.ShapeDtypeStruct((S, 2 * D), bf16),
        in_specs=[any_spec] * 8,
        out_specs=any_spec,
        scratch_shapes=[
            pltpu.VMEM((S, D), bf16),
            pltpu.VMEM((D, D), bf16),
            pltpu.VMEM((D, DH), bf16),
            pltpu.VMEM((D, DH), bf16),
            pltpu.VMEM((D, D), bf16),
            pltpu.VMEM((S, D), bf16),
            pltpu.VMEM((D, 3 * D), bf16),
            pltpu.VMEM((D, D), bf16),
            pltpu.VMEM((D, 128), bf16),
            pltpu.VMEM((4, S, 128), bf16),
            pltpu.VMEM((DH, S), bf16),
            pltpu.VMEM((S, D), bf16),
            pltpu.VMEM((D, S), f32),
            pltpu.VMEM((S, NQ), f32),
            pltpu.VMEM((S, NQ), f32),
            pltpu.VMEM((8, NQ), f32),
            pltpu.VMEM((8, NQ), f32),
            pltpu.VMEM((W + S, D), bf16),
            pltpu.VMEM((D, W + S), bf16),
            pltpu.VMEM((S, D), bf16),
            pltpu.VMEM((S, D), bf16),
            pltpu.SemaphoreType.DMA((8,)),
            pltpu.SemaphoreType.DMA((1 + S // RC,)),
        ],
        compiler_params=pltpu.CompilerParams(vmem_limit_bytes=110 * 2 ** 20),
    )(ax, A_wq, A_wk, A_wv, A_wo, bx, B_wqkv, B_wo)
    return out.reshape(1, S, 2 * D)
```

```python
import math

import jax
import jax.numpy as jnp
import jax.experimental.pallas as pl
import jax.experimental.pallas.tpu as pltpu

S = 2048
D = 1024
H = 32
DH = 32
W = 256
NQ = 512
CK = 128
RC = 512
QB = 128
KB = W + QB
NEG = -1e30
QSCALE = (DH ** -0.5) * math.log2(math.e)

f32 = jnp.float32
bf16 = jnp.bfloat16


def _nt(a, b):
    return jax.lax.dot_general(a, b, (((1,), (1,)), ((), ())),
                               preferred_element_type=f32)


def _nn(a, b):
    return jnp.dot(a, b, preferred_element_type=f32)


def _tree(x, op):
    while x.shape[0] > 8:
        h = x.shape[0] // 2
        x = op(x[:h], x[h:])
    return x


def _kernel(ax_hbm, awq_hbm, awk_hbm, awv_hbm, awo_hbm, bx_hbm, bwqkv_hbm, bwo_hbm,
            out_hbm,
            ax, awq, awk, awv, awo, bx, bwqkv, bwo,
            wkv, kpad, vt_a, q_s, ot_s, s_a, s_b, m_a, m_b,
            kb_s, vtb_s, out_a, out_b,
            in_sems, out_sems):
    srcs = (ax_hbm, awk_hbm, awv_hbm, awq_hbm, bx_hbm, bwqkv_hbm, awo_hbm, bwo_hbm)
    dsts = (ax, awk, awv, awq, bx, bwqkv, awo, bwo)
    copies = [pltpu.make_async_copy(s, d, in_sems.at[i])
              for i, (s, d) in enumerate(zip(srcs, dsts))]
    for c in copies:
        c.start()

    copies[0].wait()
    copies[1].wait()
    copies[2].wait()
    wkv[...] = jnp.zeros(wkv.shape, bf16)
    wkv[:, 0:DH] = awk[...]
    wkv[:, DH:2 * DH] = awv[...]
    lane = jax.lax.broadcasted_iota(jnp.int32, (RC, 128), 1)
    for r in range(S // RC):
        rows = slice(r * RC, (r + 1) * RC)
        kv = _nn(ax[rows, :], wkv[...])
        k_only = jnp.where(lane < DH, kv, 0.0)
        kpad[0, rows, :] = k_only.astype(bf16)
        for j in range(1, 4):
            kpad[j, rows, :] = pltpu.roll(k_only, j * DH, 1).astype(bf16)
        vt_a[:, rows] = kv.T[DH:2 * DH, :].astype(bf16)

    copies[3].wait()
    for r in range(S // RC):
        rows = slice(r * RC, (r + 1) * RC)
        q_s[rows, :] = (_nn(ax[rows, :], awq[...]) * QSCALE).astype(bf16)

    n_units = H * (S // NQ)
    n_ck = S // CK

    def get_q(u):
        t = u // H
        h = u % H
        qg = q_s[pl.ds(pl.multiple_of(t * NQ, NQ), NQ),
                 pl.ds(pl.multiple_of((h // 4) * 128, 128), 128)]
        return qg, h % 4

    def qk_chunk(qg, j, s_ref, c, m8):
        s = _nt(kpad[j, c * CK:(c + 1) * CK, :], qg)
        s_ref[c * CK:(c + 1) * CK, :] = s
        t = _tree(s, jnp.maximum)
        return t if m8 is None else jnp.maximum(m8, t)

    def sm_chunk(s_ref, c, m, l8, acc):
        p = jnp.exp2(s_ref[c * CK:(c + 1) * CK, :] - m)
        t = _tree(p, jnp.add)
        l8 = t if l8 is None else l8 + t
        o = _nn(vt_a[:, c * CK:(c + 1) * CK], p.astype(bf16))
        acc = o if acc is None else acc + o
        return l8, acc

    def step(u_next, s_next, m_next, u_cur, s_cur, m_cur):
        qg, j = get_q(u_next)
        m = m_cur[0:1, :]
        m8 = l8 = acc = None
        for c in range(n_ck):
            m8 = qk_chunk(qg, j, s_next, c, m8)
            l8, acc = sm_chunk(s_cur, c, m, l8, acc)
        m_next[...] = jnp.broadcast_to(jnp.max(m8, axis=0, keepdims=True), (8, NQ))
        t = u_cur // H
        h = u_cur % H
        l = jnp.sum(l8, axis=0, keepdims=True)
        ot_s[pl.ds(pl.multiple_of(h * DH, DH), DH),
             pl.ds(pl.multiple_of(t * NQ, NQ), NQ)] = acc / l

    qg0, j0 = get_q(0)
    m8 = None
    for c in range(n_ck):
        m8 = qk_chunk(qg0, j0, s_a, c, m8)
    m_a[...] = jnp.broadcast_to(jnp.max(m8, axis=0, keepdims=True), (8, NQ))

    def a_body(u, carry):
        un = jnp.minimum(u + 1, n_units - 1)

        @pl.when(u % 2 == 0)
        def _():
            step(un, s_b, m_b, u, s_a, m_a)

        @pl.when(u % 2 == 1)
        def _():
            step(un, s_a, m_a, u, s_b, m_b)
        return carry

    jax.lax.fori_loop(0, n_units, a_body, 0)

    copies[6].wait()
    for r in range(S // RC):
        rows = slice(r * RC, (r + 1) * RC)
        o = ot_s[:, rows].T.astype(bf16)
        out_a[rows, :] = _nn(o, awo[...]).astype(bf16)
    out_a_cp = pltpu.make_async_copy(out_a, out_hbm.at[:, 0:D], out_sems.at[0])
    out_a_cp.start()

    copies[4].wait()
    copies[5].wait()
    kb_s[0:W, :] = jnp.zeros((W, D), bf16)
    vtb_s[:, 0:W] = jnp.zeros((D, W), bf16)
    for r in range(S // RC):
        rows = slice(r * RC, (r + 1) * RC)
        prow = slice(W + r * RC, W + (r + 1) * RC)
        xr = bx[rows, :]
        q_s[rows, :] = (_nn(xr, bwqkv[:, 0:D]) * QSCALE).astype(bf16)
        kb_s[prow, :] = _nn(xr, bwqkv[:, D:2 * D]).astype(bf16)
        vtb_s[:, prow] = _nn(xr, bwqkv[:, 2 * D:3 * D]).T.astype(bf16)

    nb_units = (S // QB) * (H // 4)
    kk = jax.lax.broadcasted_iota(jnp.int32, (QB, 4 * QB), 0)
    qq = jax.lax.broadcasted_iota(jnp.int32, (QB, 4 * QB), 1) % QB
    lane_q = jax.lax.broadcasted_iota(jnp.int32, (QB, 128), 1) // DH

    def b_get_q(u):
        t = u // 8
        g = u % 8
        q0 = pl.multiple_of(t * QB, QB)
        c0 = pl.multiple_of(g * 128, 128)
        qg = q_s[pl.ds(q0, QB), pl.ds(c0, 128)]
        qm = jnp.concatenate(
            [jnp.where(lane_q == j, qg, jnp.zeros_like(qg)) for j in range(4)],
            axis=0)
        return qm, t, q0, c0

    def b_qk_chunk(qm, t, q0, c0, s_ref, c, m8):
        kg = kb_s[pl.ds(q0 + c * QB, QB), pl.ds(c0, 128)]
        s = _nt(kg, qm)
        if c == 0:
            valid = jnp.logical_and(kk > qq, t >= 2)
            s = jnp.where(valid, s, NEG)
        elif c == 1:
            s = jnp.where(t >= 1, s, NEG)
        else:
            s = jnp.where(kk <= qq, s, NEG)
        s_ref[c * QB:(c + 1) * QB, 0:4 * QB] = s
        tm = _tree(s, jnp.maximum)
        return tm if m8 is None else jnp.maximum(m8, tm)

    def b_sm_chunk(q0, c0, s_ref, c, m, l8, accs):
        p = jnp.exp2(s_ref[c * QB:(c + 1) * QB, 0:4 * QB] - m)
        tl = _tree(p, jnp.add)
        l8 = tl if l8 is None else l8 + tl
        pb = p.astype(bf16)
        new = []
        for j in range(4):
            o = _nn(vtb_s[pl.ds(c0 + j * DH, DH), pl.ds(q0 + c * QB, QB)],
                    pb[:, j * QB:(j + 1) * QB])
            new.append(o if accs is None else accs[j] + o)
        return l8, new

    def b_step(u_next, s_next, m_next, u_cur, s_cur, m_cur):
        qm, tn, q0n, c0n = b_get_q(u_next)
        q0 = pl.multiple_of((u_cur // 8) * QB, QB)
        c0 = pl.multiple_of((u_cur % 8) * 128, 128)
        m = m_cur[0:1, 0:4 * QB]
        m8 = l8 = accs = None
        for c in range(3):
            m8 = b_qk_chunk(qm, tn, q0n, c0n, s_next, c, m8)
            l8, accs = b_sm_chunk(q0, c0, s_cur, c, m, l8, accs)
        m_next[:, 0:4 * QB] = jnp.broadcast_to(
            jnp.max(m8, axis=0, keepdims=True), (8, 4 * QB))
        l = jnp.sum(l8, axis=0, keepdims=True)
        for j in range(4):
            ot_s[pl.ds(c0 + j * DH, DH), pl.ds(q0, QB)] = (
                accs[j] / l[:, j * QB:(j + 1) * QB])

    qm0, t0, q00, c00 = b_get_q(0)
    m8 = None
    for c in range(3):
        m8 = b_qk_chunk(qm0, t0, q00, c00, s_a, c, m8)
    m_a[:, 0:4 * QB] = jnp.broadcast_to(jnp.max(m8, axis=0, keepdims=True), (8, 4 * QB))

    def b_body(u, carry):
        un = jnp.minimum(u + 1, nb_units - 1)

        @pl.when(u % 2 == 0)
        def _():
            b_step(un, s_b, m_b, u, s_a, m_a)

        @pl.when(u % 2 == 1)
        def _():
            b_step(un, s_a, m_a, u, s_b, m_b)
        return carry

    jax.lax.fori_loop(0, nb_units, b_body, 0)

    copies[7].wait()
    out_b_cps = []
    for r in range(S // RC):
        rows = slice(r * RC, (r + 1) * RC)
        o = ot_s[:, rows].T.astype(bf16)
        out_b[rows, :] = _nn(o, bwo[...]).astype(bf16)
        cp = pltpu.make_async_copy(out_b.at[rows, :], out_hbm.at[rows, D:2 * D],
                                   out_sems.at[1 + r])
        cp.start()
        out_b_cps.append(cp)
    out_a_cp.wait()
    for cp in out_b_cps:
        cp.wait()


@jax.jit
def pallas_concat_heads__grouped_kv_mqa__sliding_block__prompt_kernel(
    A_x: jax.Array,
    A_wq: jax.Array,
    A_wk: jax.Array,
    A_wv: jax.Array,
    A_wo: jax.Array,
    B_x: jax.Array,
    B_wqkv: jax.Array,
    B_wo: jax.Array,
):
    ax = A_x.reshape(S, D)
    bx = B_x.reshape(S, D)
    any_spec = pl.BlockSpec(memory_space=pl.ANY)
    out = pl.pallas_call(
        _kernel,
        out_shape=jax.ShapeDtypeStruct((S, 2 * D), bf16),
        in_specs=[any_spec] * 8,
        out_specs=any_spec,
        scratch_shapes=[
            pltpu.VMEM((S, D), bf16),
            pltpu.VMEM((D, D), bf16),
            pltpu.VMEM((D, DH), bf16),
            pltpu.VMEM((D, DH), bf16),
            pltpu.VMEM((D, D), bf16),
            pltpu.VMEM((S, D), bf16),
            pltpu.VMEM((D, 3 * D), bf16),
            pltpu.VMEM((D, D), bf16),
            pltpu.VMEM((D, 128), bf16),
            pltpu.VMEM((4, S, 128), bf16),
            pltpu.VMEM((DH, S), bf16),
            pltpu.VMEM((S, D), bf16),
            pltpu.VMEM((D, S), f32),
            pltpu.VMEM((S, NQ), f32),
            pltpu.VMEM((S, NQ), f32),
            pltpu.VMEM((8, NQ), f32),
            pltpu.VMEM((8, NQ), f32),
            pltpu.VMEM((W + S, D), bf16),
            pltpu.VMEM((D, W + S), bf16),
            pltpu.VMEM((S, D), bf16),
            pltpu.VMEM((S, D), bf16),
            pltpu.SemaphoreType.DMA((8,)),
            pltpu.SemaphoreType.DMA((1 + S // RC,)),
        ],
        compiler_params=pltpu.CompilerParams(vmem_limit_bytes=110 * 2 ** 20),
    )(ax, A_wq, A_wk, A_wv, A_wo, bx, B_wqkv, B_wo)
    return out.reshape(1, S, 2 * D)
```

```python
import math

import jax
import jax.numpy as jnp
import jax.experimental.pallas as pl
import jax.experimental.pallas.tpu as pltpu

S = 2048
D = 1024
H = 32
DH = 32
W = 256
NQ = 512
CK = 128
RC = 512
QB = 128
KB = W + QB
GB = 4
NEG = -1e30
QSCALE = (DH ** -0.5) * math.log2(math.e)

f32 = jnp.float32
bf16 = jnp.bfloat16


def _nt(a, b):
    return jax.lax.dot_general(a, b, (((1,), (1,)), ((), ())),
                               preferred_element_type=f32)


def _nn(a, b):
    return jnp.dot(a, b, preferred_element_type=f32)


def _tree(x, op):
    while x.shape[0] > 8:
        h = x.shape[0] // 2
        x = op(x[:h], x[h:])
    return x


def _kernel(ax_hbm, awq_hbm, awk_hbm, awv_hbm, awo_hbm, bx_hbm, bwqkv_hbm, bwo_hbm,
            out_hbm,
            ax, awq, awk, awv, awo, bx, bwqkv, bwo,
            wkv, kpad, vt_a, q_s, ot_s, s_a, s_b, m_a, m_b,
            kb_s, vtb_s, out_a, out_b,
            in_sems, out_sems):
    srcs = (ax_hbm, awk_hbm, awv_hbm, awq_hbm, bx_hbm, bwqkv_hbm, awo_hbm, bwo_hbm)
    dsts = (ax, awk, awv, awq, bx, bwqkv, awo, bwo)
    copies = [pltpu.make_async_copy(s, d, in_sems.at[i])
              for i, (s, d) in enumerate(zip(srcs, dsts))]
    for c in copies:
        c.start()

    copies[0].wait()
    copies[1].wait()
    copies[2].wait()
    wkv[...] = jnp.zeros(wkv.shape, bf16)
    wkv[:, 0:DH] = awk[...]
    wkv[:, DH:2 * DH] = awv[...]
    lane = jax.lax.broadcasted_iota(jnp.int32, (RC, 128), 1)
    for r in range(S // RC):
        rows = slice(r * RC, (r + 1) * RC)
        kv = _nn(ax[rows, :], wkv[...])
        k_only = jnp.where(lane < DH, kv, 0.0)
        kpad[0, rows, :] = k_only.astype(bf16)
        for j in range(1, 4):
            kpad[j, rows, :] = pltpu.roll(k_only, j * DH, 1).astype(bf16)
        vt_a[:, rows] = kv.T[DH:2 * DH, :].astype(bf16)

    copies[3].wait()
    for r in range(S // RC):
        rows = slice(r * RC, (r + 1) * RC)
        q_s[rows, :] = (_nn(ax[rows, :], awq[...]) * QSCALE).astype(bf16)

    n_units = H * (S // NQ)
    n_ck = S // CK

    def get_q(u):
        t = u // H
        h = u % H
        qg = q_s[pl.ds(pl.multiple_of(t * NQ, NQ), NQ),
                 pl.ds(pl.multiple_of((h // 4) * 128, 128), 128)]
        return qg, h % 4

    def qk_chunk(qg, j, s_ref, c, m8):
        s = _nt(kpad[j, c * CK:(c + 1) * CK, :], qg)
        s_ref[c * CK:(c + 1) * CK, :] = s
        t = _tree(s, jnp.maximum)
        return t if m8 is None else jnp.maximum(m8, t)

    def sm_chunk(s_ref, c, m, l8, acc):
        p = jnp.exp2(s_ref[c * CK:(c + 1) * CK, :] - m)
        t = _tree(p, jnp.add)
        l8 = t if l8 is None else l8 + t
        o = _nn(vt_a[:, c * CK:(c + 1) * CK], p.astype(bf16))
        acc = o if acc is None else acc + o
        return l8, acc

    def step(u_next, s_next, m_next, u_cur, s_cur, m_cur):
        qg, j = get_q(u_next)
        m = m_cur[0:1, :]
        m8 = l8 = acc = None
        for c in range(n_ck):
            m8 = qk_chunk(qg, j, s_next, c, m8)
            l8, acc = sm_chunk(s_cur, c, m, l8, acc)
        m_next[...] = jnp.broadcast_to(jnp.max(m8, axis=0, keepdims=True), (8, NQ))
        t = u_cur // H
        h = u_cur % H
        l = jnp.sum(l8, axis=0, keepdims=True)
        ot_s[pl.ds(pl.multiple_of(h * DH, DH), DH),
             pl.ds(pl.multiple_of(t * NQ, NQ), NQ)] = acc / l

    qg0, j0 = get_q(0)
    m8 = None
    for c in range(n_ck):
        m8 = qk_chunk(qg0, j0, s_a, c, m8)
    m_a[...] = jnp.broadcast_to(jnp.max(m8, axis=0, keepdims=True), (8, NQ))

    def a_body(u, carry):
        un = jnp.minimum(u + 1, n_units - 1)

        @pl.when(u % 2 == 0)
        def _():
            step(un, s_b, m_b, u, s_a, m_a)

        @pl.when(u % 2 == 1)
        def _():
            step(un, s_a, m_a, u, s_b, m_b)
        return carry

    jax.lax.fori_loop(0, n_units, a_body, 0)

    copies[6].wait()
    for r in range(S // RC):
        rows = slice(r * RC, (r + 1) * RC)
        o = ot_s[:, rows].T.astype(bf16)
        out_a[rows, :] = _nn(o, awo[...]).astype(bf16)
    out_a_cp = pltpu.make_async_copy(out_a, out_hbm.at[:, 0:D], out_sems.at[0])
    out_a_cp.start()

    copies[4].wait()
    copies[5].wait()
    kb_s[0:W, :] = jnp.zeros((W, D), bf16)
    vtb_s[:, 0:W] = jnp.zeros((D, W), bf16)
    for r in range(S // RC):
        rows = slice(r * RC, (r + 1) * RC)
        prow = slice(W + r * RC, W + (r + 1) * RC)
        xr = bx[rows, :]
        q_s[rows, :] = (_nn(xr, bwqkv[:, 0:D]) * QSCALE).astype(bf16)
        kb_s[prow, :] = _nn(xr, bwqkv[:, D:2 * D]).astype(bf16)
        vtb_s[:, prow] = _nn(xr, bwqkv[:, 2 * D:3 * D]).T.astype(bf16)

    upt = (H // 4) // GB
    nb_units = (S // QB) * upt
    kk = jax.lax.broadcasted_iota(jnp.int32, (QB, 4 * QB), 0)
    qq = jax.lax.broadcasted_iota(jnp.int32, (QB, 4 * QB), 1) % QB
    lane_q = jax.lax.broadcasted_iota(jnp.int32, (QB, 128), 1) // DH

    def b_pos(u, gi):
        t = u // upt
        q0 = pl.multiple_of(t * QB, QB)
        c0 = pl.multiple_of(((u % upt) * GB + gi) * 128, 128)
        return t, q0, c0

    def b_get_q(q0, c0):
        qg = q_s[pl.ds(q0, QB), pl.ds(c0, 128)]
        return jnp.concatenate(
            [jnp.where(lane_q == j, qg, jnp.zeros_like(qg)) for j in range(4)],
            axis=0)

    def b_qk_chunk(qm, t, q0, c0, s_ref, gi, c, m8):
        kg = kb_s[pl.ds(q0 + c * QB, QB), pl.ds(c0, 128)]
        s = _nt(kg, qm)
        if c == 0:
            valid = jnp.logical_and(kk > qq, t >= 2)
            s = jnp.where(valid, s, NEG)
        elif c == 1:
            s = jnp.where(t >= 1, s, NEG)
        else:
            s = jnp.where(kk <= qq, s, NEG)
        r0 = gi * KB + c * QB
        s_ref[r0:r0 + QB, 0:4 * QB] = s
        tm = _tree(s, jnp.maximum)
        return tm if m8 is None else jnp.maximum(m8, tm)

    def b_sm_chunk(q0, c0, s_ref, gi, c, m, l8, accs):
        r0 = gi * KB + c * QB
        p = jnp.exp2(s_ref[r0:r0 + QB, 0:4 * QB] - m)
        tl = _tree(p, jnp.add)
        l8 = tl if l8 is None else l8 + tl
        pb = p.astype(bf16)
        new = []
        for j in range(4):
            o = _nn(vtb_s[pl.ds(c0 + j * DH, DH), pl.ds(q0 + c * QB, QB)],
                    pb[:, j * QB:(j + 1) * QB])
            new.append(o if accs is None else accs[j] + o)
        return l8, new

    def b_step(u_next, s_next, m_next, u_cur, s_cur, m_cur):
        for gi in range(GB):
            if u_next is not None:
                tn, q0n, c0n = b_pos(u_next, gi)
                qm = b_get_q(q0n, c0n)
            if u_cur is not None:
                _, q0, c0 = b_pos(u_cur, gi)
                m = m_cur[gi:gi + 1, 0:4 * QB]
            m8 = l8 = accs = None
            for c in range(3):
                if u_next is not None:
                    m8 = b_qk_chunk(qm, tn, q0n, c0n, s_next, gi, c, m8)
                if u_cur is not None:
                    l8, accs = b_sm_chunk(q0, c0, s_cur, gi, c, m, l8, accs)
            if u_next is not None:
                m_next[gi:gi + 1, 0:4 * QB] = jnp.max(m8, axis=0, keepdims=True)
            if u_cur is not None:
                l = jnp.sum(l8, axis=0, keepdims=True)
                for j in range(4):
                    ot_s[pl.ds(c0 + j * DH, DH), pl.ds(q0, QB)] = (
                        accs[j] / l[:, j * QB:(j + 1) * QB])

    b_step(0, s_a, m_a, None, None, None)

    def b_body(u, carry):
        un = jnp.minimum(u + 1, nb_units - 1)

        @pl.when(u % 2 == 0)
        def _():
            b_step(un, s_b, m_b, u, s_a, m_a)

        @pl.when(u % 2 == 1)
        def _():
            b_step(un, s_a, m_a, u, s_b, m_b)
        return carry

    jax.lax.fori_loop(0, nb_units, b_body, 0)

    copies[7].wait()
    out_b_cps = []
    for r in range(S // RC):
        rows = slice(r * RC, (r + 1) * RC)
        o = ot_s[:, rows].T.astype(bf16)
        out_b[rows, :] = _nn(o, bwo[...]).astype(bf16)
        cp = pltpu.make_async_copy(out_b.at[rows, :], out_hbm.at[rows, D:2 * D],
                                   out_sems.at[1 + r])
        cp.start()
        out_b_cps.append(cp)
    out_a_cp.wait()
    for cp in out_b_cps:
        cp.wait()


@jax.jit
def pallas_concat_heads__grouped_kv_mqa__sliding_block__prompt_kernel(
    A_x: jax.Array,
    A_wq: jax.Array,
    A_wk: jax.Array,
    A_wv: jax.Array,
    A_wo: jax.Array,
    B_x: jax.Array,
    B_wqkv: jax.Array,
    B_wo: jax.Array,
):
    ax = A_x.reshape(S, D)
    bx = B_x.reshape(S, D)
    any_spec = pl.BlockSpec(memory_space=pl.ANY)
    out = pl.pallas_call(
        _kernel,
        out_shape=jax.ShapeDtypeStruct((S, 2 * D), bf16),
        in_specs=[any_spec] * 8,
        out_specs=any_spec,
        scratch_shapes=[
            pltpu.VMEM((S, D), bf16),
            pltpu.VMEM((D, D), bf16),
            pltpu.VMEM((D, DH), bf16),
            pltpu.VMEM((D, DH), bf16),
            pltpu.VMEM((D, D), bf16),
            pltpu.VMEM((S, D), bf16),
            pltpu.VMEM((D, 3 * D), bf16),
            pltpu.VMEM((D, D), bf16),
            pltpu.VMEM((D, 128), bf16),
            pltpu.VMEM((4, S, 128), bf16),
            pltpu.VMEM((DH, S), bf16),
            pltpu.VMEM((S, D), bf16),
            pltpu.VMEM((D, S), f32),
            pltpu.VMEM((S, NQ), f32),
            pltpu.VMEM((S, NQ), f32),
            pltpu.VMEM((8, NQ), f32),
            pltpu.VMEM((8, NQ), f32),
            pltpu.VMEM((W + S, D), bf16),
            pltpu.VMEM((D, W + S), bf16),
            pltpu.VMEM((S, D), bf16),
            pltpu.VMEM((S, D), bf16),
            pltpu.SemaphoreType.DMA((8,)),
            pltpu.SemaphoreType.DMA((1 + S // RC,)),
        ],
        compiler_params=pltpu.CompilerParams(vmem_limit_bytes=110 * 2 ** 20),
    )(ax, A_wq, A_wk, A_wv, A_wo, bx, B_wqkv, B_wo)
    return out.reshape(1, S, 2 * D)
```

```python
import math

import jax
import jax.numpy as jnp
import jax.experimental.pallas as pl
import jax.experimental.pallas.tpu as pltpu

S = 2048
D = 1024
H = 32
DH = 32
W = 256
NQ = 512
CK = 128
UA = 4
RC = 512
WC = 256
QB = 128
KB = W + QB
TB = 2
NEG = -1e30
QSCALE = (DH ** -0.5) * math.log2(math.e)

f32 = jnp.float32
bf16 = jnp.bfloat16


def _nt(a, b):
    return jax.lax.dot_general(a, b, (((1,), (1,)), ((), ())),
                               preferred_element_type=f32)


def _nn(a, b):
    return jnp.dot(a, b, preferred_element_type=f32)


def _tree(x, op):
    while x.shape[0] > 8:
        h = x.shape[0] // 2
        x = op(x[:h], x[h:])
    return x


def _kernel(ax_hbm, awq_hbm, awk_hbm, awv_hbm, awo_hbm, bx_hbm, bwqkv_hbm, bwo_hbm,
            out_hbm,
            ax, awq, awk, awv, awo, bx, bwqkv, bwo,
            wkv, kpad, vt_a, q_s, ot_s, s_a, s_b, m_a, m_b,
            kb_s, vtb_s, bias_s,
            in_sems, out_sems):
    n_rc = S // RC
    out_a = ax
    out_b = bx
    ax_cps = [pltpu.make_async_copy(ax_hbm.at[r * RC:(r + 1) * RC, :],
                                    ax.at[r * RC:(r + 1) * RC, :], in_sems.at[r])
              for r in range(n_rc)]
    srcs = (awk_hbm, awv_hbm, bx_hbm, bwqkv_hbm, awo_hbm, bwo_hbm)
    dsts = (awk, awv, bx, bwqkv, awo, bwo)
    copies = [pltpu.make_async_copy(s, d, in_sems.at[n_rc + i])
              for i, (s, d) in enumerate(zip(srcs, dsts))]
    cp_awk, cp_awv, cp_bx, cp_bwqkv, cp_awo, cp_bwo = copies
    n_wc = D // WC
    awq_cps = [pltpu.make_async_copy(awq_hbm.at[:, c * WC:(c + 1) * WC],
                                     awq.at[:, c * WC:(c + 1) * WC],
                                     in_sems.at[n_rc + 6 + c])
               for c in range(n_wc)]
    ax_cps[0].start()
    for c in range(n_wc):
        awq_cps[c].start()

    ax_cps[0].wait()
    for c in range(n_wc):
        cols = slice(c * WC, (c + 1) * WC)
        awq_cps[c].wait()
        if c == 1:
            for r in range(1, n_rc):
                ax_cps[r].start()
            cp_awk.start()
            cp_awv.start()
        q_s[0:RC, cols] = (_nn(ax[0:RC, :], awq[:, cols]) * QSCALE).astype(bf16)

    def aq_body(r, carry):
        rows = pl.ds(pl.multiple_of(r * RC, RC), RC)
        pltpu.make_async_copy(ax_hbm.at[rows, :], ax.at[rows, :], in_sems.at[r]).wait()

        @pl.when(r == n_rc - 1)
        def _():
            cp_bx.start()
            cp_bwqkv.start()
            cp_awo.start()
            cp_bwo.start()
        q_s[rows, :] = (_nn(ax[rows, :], awq[...]) * QSCALE).astype(bf16)
        return carry

    jax.lax.fori_loop(1, n_rc, aq_body, 0)

    cp_awk.wait()
    cp_awv.wait()
    wkv[0:DH, :] = awk[...]
    wkv[DH:2 * DH, :] = awv[...]
    wkv[2 * DH:128, :] = jnp.zeros((128 - 2 * DH, D), bf16)
    lane = jax.lax.broadcasted_iota(jnp.int32, (RC, 128), 1)
    for r in range(n_rc):
        rows = slice(r * RC, (r + 1) * RC)
        kv = _nt(ax[rows, :], wkv[...])
        k_only = jnp.where(lane < DH, kv, 0.0)
        kpad[0, rows, :] = k_only.astype(bf16)
        for j in range(1, 4):
            kpad[j, rows, :] = pltpu.roll(k_only, j * DH, 1).astype(bf16)
        vt_a[:, rows] = kv.T[DH:2 * DH, :].astype(bf16)

    assert UA == 4
    n_g = H // 4
    n_steps = n_g * (S // NQ)
    n_ck = S // CK

    def a_pos(i):
        t0 = pl.multiple_of((i // n_g) * NQ, NQ)
        c0 = pl.multiple_of((i % n_g) * 128, 128)
        return t0, c0

    def qk_chunk(qg, j, s_ref, k, c, m8):
        s = _nt(kpad[j, c * CK:(c + 1) * CK, :], qg)
        s_ref[k * S + c * CK:k * S + (c + 1) * CK, :] = s
        t = _tree(s, jnp.maximum)
        return t if m8 is None else jnp.maximum(m8, t)

    def sm_chunk(s_ref, k, c, m, l8, acc):
        p = jnp.exp2(s_ref[k * S + c * CK:k * S + (c + 1) * CK, :] - m)
        t = _tree(p, jnp.add)
        l8 = t if l8 is None else l8 + t
        o = _nn(vt_a[:, c * CK:(c + 1) * CK], p.astype(bf16))
        acc = o if acc is None else acc + o
        return l8, acc

    def step(i_next, s_next, m_next, i_cur, s_cur, m_cur):
        if i_next is not None:
            t0n, c0n = a_pos(i_next)
            qg = q_s[pl.ds(t0n, NQ), pl.ds(c0n, 128)]
        if i_cur is not None:
            t0, c0 = a_pos(i_cur)
        for k in range(UA):
            if i_cur is not None:
                m = m_cur[k:k + 1, :]
            m8 = l8 = acc = None
            for c in range(n_ck):
                if i_next is not None:
                    m8 = qk_chunk(qg, k, s_next, k, c, m8)
                if i_cur is not None:
                    l8, acc = sm_chunk(s_cur, k, c, m, l8, acc)
            if i_next is not None:
                m_next[k:k + 1, :] = jnp.max(m8, axis=0, keepdims=True)
            if i_cur is not None:
                l = jnp.sum(l8, axis=0, keepdims=True)
                ot_s[pl.ds(c0 + k * DH, DH), pl.ds(t0, NQ)] = acc / l

    step(0, s_a, m_a, None, None, None)

    def a_body(i, carry):
        @pl.when(i % 2 == 0)
        def _():
            step(i + 1, s_b, m_b, i, s_a, m_a)

        @pl.when(i % 2 == 1)
        def _():
            step(i + 1, s_a, m_a, i, s_b, m_b)
        return carry

    jax.lax.fori_loop(0, n_steps - 1, a_body, 0)
    assert n_steps % 2 == 0
    step(None, None, None, n_steps - 1, s_b, m_b)

    cp_awo.wait()

    def ao_body(r, carry):
        rows = pl.ds(pl.multiple_of(r * RC, RC), RC)
        o = ot_s[:, rows].T.astype(bf16)
        out_a[rows, :] = _nn(o, awo[...]).astype(bf16)
        return carry

    jax.lax.fori_loop(0, n_rc, ao_body, 0)
    out_a_cp = pltpu.make_async_copy(out_a, out_hbm.at[:, 0:D], out_sems.at[0])
    out_a_cp.start()

    cp_bx.wait()
    cp_bwqkv.wait()
    kb_s[0:W, :] = jnp.zeros((W, D), bf16)
    vtb_s[:, 0:W] = jnp.zeros((D, W), bf16)

    def bqkv_body(r, carry):
        rows = pl.ds(pl.multiple_of(r * RC, RC), RC)
        prow = pl.ds(pl.multiple_of(W + r * RC, 128), RC)
        xr = bx[rows, :]
        q_s[rows, :] = (_nn(xr, bwqkv[:, 0:D]) * QSCALE).astype(bf16)
        kb_s[prow, :] = _nn(xr, bwqkv[:, D:2 * D]).astype(bf16)
        vtb_s[:, prow] = _nn(xr, bwqkv[:, 2 * D:3 * D]).T.astype(bf16)
        return carry

    jax.lax.fori_loop(0, n_rc, bqkv_body, 0)

    nb_steps = S // QB // TB
    kk = jax.lax.broadcasted_iota(jnp.int32, (QB, 4 * QB), 0)
    qq = jax.lax.broadcasted_iota(jnp.int32, (QB, 4 * QB), 1) % QB
    lane_q = jax.lax.broadcasted_iota(jnp.int32, (QB, 128), 1) // DH
    bias_s[0] = jnp.where(kk > qq, 0.0, NEG)
    bias_s[1] = jnp.where(kk <= qq, 0.0, NEG)

    def b_q0(i, gi):
        t = i * TB + gi // n_g
        if isinstance(t, int):
            return t * QB
        return pl.multiple_of(t * QB, QB)

    def b_get_q(q0, c0):
        qg = q_s[pl.ds(q0, QB), c0:c0 + 128]
        return jnp.concatenate(
            [jnp.where(lane_q == j, qg, jnp.zeros_like(qg)) for j in range(4)],
            axis=0)

    def b_qk_chunk(qm, q0, c0, s_ref, gi, c, m8):
        if isinstance(q0, int) and q0 + c * QB < W:
            s = jnp.full((QB, 4 * QB), NEG, f32)
        else:
            kg = kb_s[pl.ds(q0 + c * QB, QB), c0:c0 + 128]
            s = _nt(kg, qm)
            if c == 0:
                s = s + bias_s[0]
            elif c == 2:
                s = s + bias_s[1]
        r0 = gi * KB + c * QB
        s_ref[r0:r0 + QB, 0:4 * QB] = s
        tm = _tree(s, jnp.maximum)
        return tm if m8 is None else jnp.maximum(m8, tm)

    def b_sm_chunk(q0, c0, s_ref, gi, c, m, l8, accs):
        r0 = gi * KB + c * QB
        p = jnp.exp2(s_ref[r0:r0 + QB, 0:4 * QB] - m)
        tl = _tree(p, jnp.add)
        l8 = tl if l8 is None else l8 + tl
        pb = p.astype(bf16)
        new = []
        for j in range(4):
            o = _nn(vtb_s[c0 + j * DH:c0 + (j + 1) * DH, pl.ds(q0 + c * QB, QB)],
                    pb[:, j * QB:(j + 1) * QB])
            new.append(o if accs is None else accs[j] + o)
        return l8, new

    def b_step(i_next, s_next, m_next, i_cur, s_cur, m_cur):
        for gi in range(TB * n_g):
            c0 = (gi % n_g) * 128
            if i_next is not None:
                q0n = b_q0(i_next, gi)
                qm = b_get_q(q0n, c0)
            if i_cur is not None:
                q0 = b_q0(i_cur, gi)
                m = m_cur[gi:gi + 1, 0:4 * QB]
            m8 = l8 = accs = None
            for c in range(3):
                if i_next is not None:
                    m8 = b_qk_chunk(qm, q0n, c0, s_next, gi, c, m8)
                if i_cur is not None:
                    l8, accs = b_sm_chunk(q0, c0, s_cur, gi, c, m, l8, accs)
            if i_next is not None:
                m_next[gi:gi + 1, 0:4 * QB] = jnp.max(m8, axis=0, keepdims=True)
            if i_cur is not None:
                l = jnp.sum(l8, axis=0, keepdims=True)
                for j in range(4):
                    ot_s[c0 + j * DH:c0 + (j + 1) * DH, pl.ds(q0, QB)] = (
                        accs[j] / l[:, j * QB:(j + 1) * QB])

    assert TB * QB >= W
    b_step(0, s_a, m_a, None, None, None)

    def b_body(i, carry):
        @pl.when(i % 2 == 0)
        def _():
            b_step(i + 1, s_b, m_b, i, s_a, m_a)

        @pl.when(i % 2 == 1)
        def _():
            b_step(i + 1, s_a, m_a, i, s_b, m_b)
        return carry

    jax.lax.fori_loop(0, nb_steps - 1, b_body, 0)
    assert nb_steps % 2 == 0
    b_step(None, None, None, nb_steps - 1, s_b, m_b)

    cp_bwo.wait()

    def bo_body(r, carry):
        rows = pl.ds(pl.multiple_of(r * RC, RC), RC)
        o = ot_s[:, rows].T.astype(bf16)
        out_b[rows, :] = _nn(o, bwo[...]).astype(bf16)
        pltpu.make_async_copy(out_b.at[rows, :], out_hbm.at[rows, D:2 * D],
                              out_sems.at[1 + r]).start()
        return carry

    jax.lax.fori_loop(0, n_rc, bo_body, 0)
    out_a_cp.wait()
    for r in range(n_rc):
        rows = slice(r * RC, (r + 1) * RC)
        pltpu.make_async_copy(out_b.at[rows, :], out_hbm.at[rows, D:2 * D],
                              out_sems.at[1 + r]).wait()


@jax.jit
def pallas_concat_heads__grouped_kv_mqa__sliding_block__prompt_kernel(
    A_x: jax.Array,
    A_wq: jax.Array,
    A_wk: jax.Array,
    A_wv: jax.Array,
    A_wo: jax.Array,
    B_x: jax.Array,
    B_wqkv: jax.Array,
    B_wo: jax.Array,
):
    ax = A_x.reshape(S, D)
    bx = B_x.reshape(S, D)
    any_spec = pl.BlockSpec(memory_space=pl.ANY)
    out = pl.pallas_call(
        _kernel,
        out_shape=jax.ShapeDtypeStruct((S, 2 * D), bf16),
        in_specs=[any_spec] * 8,
        out_specs=any_spec,
        scratch_shapes=[
            pltpu.VMEM((S, D), bf16),
            pltpu.VMEM((D, D), bf16),
            pltpu.VMEM((DH, D), bf16),
            pltpu.VMEM((DH, D), bf16),
            pltpu.VMEM((D, D), bf16),
            pltpu.VMEM((S, D), bf16),
            pltpu.VMEM((D, 3 * D), bf16),
            pltpu.VMEM((D, D), bf16),
            pltpu.VMEM((128, D), bf16),
            pltpu.VMEM((4, S, 128), bf16),
            pltpu.VMEM((DH, S), bf16),
            pltpu.VMEM((S, D), bf16),
            pltpu.VMEM((D, S), f32),
            pltpu.VMEM((max(UA * S, TB * (H // 4) * KB), NQ), f32),
            pltpu.VMEM((max(UA * S, TB * (H // 4) * KB), NQ), f32),
            pltpu.VMEM((max(8, TB * (H // 4)), NQ), f32),
            pltpu.VMEM((max(8, TB * (H // 4)), NQ), f32),
            pltpu.VMEM((W + S, D), bf16),
            pltpu.VMEM((D, W + S), bf16),
            pltpu.VMEM((2, QB, 4 * QB), f32),
            pltpu.SemaphoreType.DMA((6 + S // RC + D // WC,)),
            pltpu.SemaphoreType.DMA((1 + S // RC,)),
        ],
        compiler_params=pltpu.CompilerParams(vmem_limit_bytes=110 * 2 ** 20),
    )(ax, A_wq, A_wk.T, A_wv.T, A_wo, bx, B_wqkv, B_wo)
    return out.reshape(1, S, 2 * D)
```
